```python
import os as _os
_os.environ.setdefault('JAX_PLATFORMS', 'cpu')
import jax
import jax.numpy as jnp

def _softmax(x, axis=-1):
    return jax.nn.softmax(x, axis=axis)

def _gelu(x):
    return jax.nn.gelu(x, approximate=True)

def _silu(x):
    return jax.nn.silu(x)

def _sigmoid(x):
    return jax.nn.sigmoid(x)

def _layernorm(x, axis=-1, eps=1e-05):
    m = jnp.mean(x, axis=axis, keepdims=True)
    v = jnp.var(x, axis=axis, keepdims=True)
    return (x - m) / jnp.sqrt(v + eps)

def _scatter_add(tgt, idx, src, axis=0):
    return tgt.at[idx].add(src)

def _segment_sum(src, seg, n):
    return jax.ops.segment_sum(src, seg, n)

class _Rng:

    def __init__(self, key):
        self._k = key

    def _next(self):
        self._k, sub = jax.random.split(self._k)
        return sub

    def normal(self, shape):
        return jax.random.normal(self._next(), shape, dtype=jnp.bfloat16)

    def randint(self, lo, hi, shape):
        return jax.random.randint(self._next(), shape, lo, hi, dtype=jnp.int32)

    def uniform(self, shape, lo=0.0, hi=1.0):
        return jax.random.uniform(self._next(), shape, jnp.bfloat16, lo, hi)

    def permutation(self, n):
        return jax.random.permutation(self._next(), n)
kernel_name = 'adaLN_cond__mha_block__dense_activation_squared_relu__prompt'

def setup_inputs():
    _rng = _Rng(jax.random.key(int.from_bytes(__import__("os").urandom(4), "little")))
    _w = lambda a: (lambda t: t.astype(jnp.bfloat16) if jnp.issubdtype(t.dtype, jnp.floating) else t)(jnp.asarray(a))

    def _A_setup():
        B, S, D, H = (1, 2048, 512, 32)
        return {'x': _w((lambda *s: _rng.normal(s) * 0.05)(B, S, D)), 'wqkv': _w((lambda *s: _rng.normal(s) * 0.1)(D, 3 * D)), 'wo': _w((lambda *s: _rng.normal(s) * 0.05)(D, D))}
    _A_in = _A_setup()

    def _B_setup():
        B, S, D, F = (1, 2048, 512, 1792)
        return {'x': _w((lambda *s: _rng.normal(s) * 0.05)(B, S, D)), 'w1': _w((lambda *s: _rng.normal(s) * 0.05)(D, F)), 'b1': _w((lambda *s: _rng.normal(s) * 0.05)(F)), 'w2': _w((lambda *s: _rng.normal(s) * 0.05)(F, D)), 'b2': _w((lambda *s: _rng.normal(s) * 0.05)(D))}
    _B_in = _B_setup()
    return {'A_x': _A_in['x'], 'A_wqkv': _A_in['wqkv'], 'A_wo': _A_in['wo'], 'B_x': _B_in['x'], 'B_w1': _B_in['w1'], 'B_b1': _B_in['b1'], 'B_w2': _B_in['w2'], 'B_b2': _B_in['b2'], 'c': _w((lambda *s: _rng.normal(s) * 0.05)(1, 512) * 8.0), 'w_mod': _w((lambda *s: _rng.normal(s) * 0.05)(512, 6 * 512) * 512 ** (-0.5) * 8.0)}

def reference(A_x, A_wqkv, A_wo, B_x, B_w1, B_b1, B_w2, B_b2, c, w_mod):

    def _A_ref(x, wqkv, wo):
        B, S, D = x.shape
        H = 32
        Dh = D // H
        qkv = (lambda x, *d: x.transpose(*d))((x @ wqkv).reshape(B, S, 3, H, Dh), 2, 0, 3, 1, 4)
        q, k, v = (qkv[0], qkv[1], qkv[2])
        scores = jnp.einsum('bhqd,bhkd->bhqk', q, k) * Dh ** (-0.5)
        p = _softmax(scores, axis=-1)
        o = jnp.einsum('bhqk,bhkd->bhqd', p, v)
        return (lambda x, *d: x.transpose(*d))(o, 0, 2, 1, 3).reshape(B, S, D) @ wo

    def _B_ref(x, w1, b1, w2, b2):
        h = jnp.einsum('bsd,df->bsf', x, w1) + b1
        zero = jnp.zeros_like(h)
        r = jnp.where(h > zero, h, zero)
        h = r * r
        out = jnp.einsum('bsf,fd->bsd', h, w2) + b2
        return out
    x = A_x
    mod = (_silu(c) @ w_mod).reshape(c.shape[0], 6, 1, -1)
    sa, ca, ga, sb, cb, gb = (mod[:, 0].copy(), mod[:, 1].copy(), mod[:, 2].copy(), mod[:, 3].copy(), mod[:, 4].copy(), mod[:, 5].copy())
    h = _layernorm(x, axis=-1) * (1 + ca) + sa
    x = x + ga * _A_ref(h, A_wqkv, A_wo)
    h = _layernorm(x, axis=-1) * (1 + cb) + sb
    x = x + gb * _B_ref(h, B_w1, B_b1, B_w2, B_b2)
    return x
```

```python
import jax
import jax.numpy as jnp
import jax.experimental.pallas as pl
import jax.experimental.pallas.tpu as pltpu

S = 2048
D = 512
H = 32
DH = 16
F = 1792
EPS = 1e-5

LOG2E = 1.4426950408889634
QSCALE = (DH ** -0.5) * LOG2E

TQ = 512
CK = 128
UPB = 4
PIPE = 2
NQ = S // TQ
NU = H * NQ
NC = S // CK

RB = 512

LSUM_MIN = 2.0 ** -80

_NT = (((1,), (1,)), ((), ()))


def _layernorm(x):
    mu = jnp.mean(x, axis=-1, keepdims=True)
    xc = x - mu
    var = jnp.mean(xc * xc, axis=-1, keepdims=True)
    return xc * jax.lax.rsqrt(var + EPS)


def _kernel(x_ref, wqkv_ref, wo_ref, w1_ref, b1_ref, w2_ref, b2_ref, c_ref, wmod_ref,
            o_ref,
            k_scr, qt_scr, vt_scr, ot_scr, mb_scr, mod_scr):
    f32 = jnp.float32
    bf16 = jnp.bfloat16

    c = c_ref[...].astype(f32)
    sc = c * jax.nn.sigmoid(c)
    sc8 = jnp.broadcast_to(sc, (8, D)).astype(bf16)
    mod_scr[...] = jnp.dot(sc8, wmod_ref[...], preferred_element_type=f32)

    sa = mod_scr[0:1, 0 * D:1 * D]
    ca = mod_scr[0:1, 1 * D:2 * D]

    wq_t = wqkv_ref[:, 0:D].astype(f32).T.astype(bf16)
    wv_t = wqkv_ref[:, 2 * D:3 * D].astype(f32).T.astype(bf16)
    gi = jax.lax.broadcasted_iota(jnp.int32, (H, D), 0)
    gj = jax.lax.broadcasted_iota(jnp.int32, (H, D), 1)
    gmat = jnp.where((gj // DH) == gi, 1.0, 0.0).astype(bf16)

    k2max = None
    q2_parts = []
    for rb in range(S // RB):
        rows = slice(rb * RB, (rb + 1) * RB)
        xb = x_ref[rows, :].astype(f32)
        hb = (_layernorm(xb) * (1.0 + ca) + sa).astype(bf16)
        kb = jnp.dot(hb, wqkv_ref[:, D:2 * D], preferred_element_type=f32).astype(bf16)
        k_scr[rows, :] = kb
        qtb = (jax.lax.dot_general(wq_t, hb, _NT, preferred_element_type=f32) * QSCALE).astype(bf16)
        qt_scr[:, rows] = qtb
        vt_scr[:, rows] = jax.lax.dot_general(wv_t, hb, _NT, preferred_element_type=f32).astype(bf16)
        kf = kb.astype(f32)
        k2 = jax.lax.dot_general(gmat, (kf * kf).astype(bf16), _NT, preferred_element_type=f32)
        k2m = jnp.max(k2, axis=1, keepdims=True)
        k2max = k2m if k2max is None else jnp.maximum(k2max, k2m)
        qf = qtb.astype(f32)
        q2_parts.append(jnp.dot(gmat, (qf * qf).astype(bf16), preferred_element_type=f32))
    for rb in range(S // RB):
        mb = jnp.sqrt(q2_parts[rb] * k2max) * (1.0 + 2.0 ** -6)
        for h in range(H):
            mb_scr[h, :, rb * RB:(rb + 1) * RB] = jnp.broadcast_to(mb[h:h + 1, :], (8, RB))

    def masked_q(u, tq):
        nq = S // tq
        h = u // nq
        g = h // 8
        hh = h % 8
        goff = pl.multiple_of(g * 128, 128)
        qoff = pl.multiple_of((u % nq) * tq, tq)
        qt = qt_scr[pl.ds(goff, 128), pl.ds(qoff, tq)]
        row = jax.lax.broadcasted_iota(jnp.int32, (128, tq), 0)
        qm = jnp.where((row // DH) == hh, qt, jnp.zeros_like(qt))
        return h, goff, qoff, qm

    def unit_info(u):
        h, goff, qoff, qm = masked_q(u, TQ)
        m8 = mb_scr[h, :, pl.ds(qoff, TQ)]
        return goff, qm, m8

    def qk(c, goff, qm):
        kg = k_scr[c * CK:(c + 1) * CK, pl.ds(goff, 128)]
        return jnp.dot(kg, qm, preferred_element_type=f32)

    def softmax_pv(c, u, st, m8, acc, l):
        hoff = pl.multiple_of((u // NQ) * DH, DH)
        p = jnp.exp2(st.reshape(CK // 8, 8, TQ) - m8[None])
        ls = jnp.sum(p, axis=0)
        vt = vt_scr[pl.ds(hoff, DH), c * CK:(c + 1) * CK]
        ot = jnp.dot(vt, p.reshape(CK, TQ).astype(bf16), preferred_element_type=f32)
        return (ot if acc is None else acc + ot), (ls if l is None else l + ls)

    def finish(u, acc, l, lmin):
        hoff = pl.multiple_of((u // NQ) * DH, DH)
        qoff = pl.multiple_of((u % NQ) * TQ, TQ)
        lt = jnp.sum(l, axis=0, keepdims=True)
        ot_scr[pl.ds(hoff, DH), pl.ds(qoff, TQ)] = (acc / lt).astype(bf16)
        return jnp.minimum(lmin, lt)

    def attn_body(j, lmin):
        tiles = [(i, c) for i in range(UPB) for c in range(NC)]
        info = [unit_info(j * UPB + i) for i in range(UPB)]
        sts = {}
        accs = {i: (None, None) for i in range(UPB)}
        n = len(tiles)
        for t in range(n + PIPE):
            if t < n:
                i, c = tiles[t]
                sts[t] = qk(c, info[i][0], info[i][1])
            if t >= PIPE:
                i, c = tiles[t - PIPE]
                acc, l = accs[i]
                accs[i] = softmax_pv(c, j * UPB + i, sts.pop(t - PIPE), info[i][2], acc, l)
                if c == NC - 1:
                    lmin = finish(j * UPB + i, accs[i][0], accs[i][1], lmin)
        return lmin

    lmin = jax.lax.fori_loop(0, NU // UPB, attn_body, jnp.full((1, TQ), jnp.inf, f32))
    safe = jnp.min(lmin) >= LSUM_MIN

    @pl.when(jnp.logical_not(safe))
    def _():
        tq = 128

        def exact_body(u, carry):
            h, goff, qoff, qm = masked_q(u, tq)
            hoff = pl.multiple_of(h * DH, DH)
            st = jnp.dot(k_scr[:, pl.ds(goff, 128)], qm, preferred_element_type=f32)
            m = jnp.max(st, axis=0, keepdims=True)
            p = jnp.exp2(st - m)
            lt = jnp.sum(p, axis=0, keepdims=True)
            ot = jnp.dot(vt_scr[pl.ds(hoff, DH), :], p.astype(bf16), preferred_element_type=f32)
            ot_scr[pl.ds(hoff, DH), pl.ds(qoff, tq)] = (ot / lt).astype(bf16)
            return carry

        jax.lax.fori_loop(0, H * (S // tq), exact_body, 0)

    ga = mod_scr[0:1, 2 * D:3 * D]
    sb = mod_scr[0:1, 3 * D:4 * D]
    cb = mod_scr[0:1, 4 * D:5 * D]
    gb = mod_scr[0:1, 5 * D:6 * D]
    b1 = b1_ref[...].astype(f32)
    b2 = b2_ref[...].astype(f32)
    for rb in range(S // RB):
        rows = slice(rb * RB, (rb + 1) * RB)
        ob = ot_scr[:, rows].astype(f32).T.astype(bf16)
        attn = jnp.dot(ob, wo_ref[...], preferred_element_type=f32)
        x1 = x_ref[rows, :].astype(f32) + ga * attn
        h2 = (_layernorm(x1) * (1.0 + cb) + sb).astype(bf16)
        a = jnp.dot(h2, w1_ref[...], preferred_element_type=f32) + b1
        r = jnp.maximum(a, 0.0)
        a2 = (r * r).astype(bf16)
        y = jnp.dot(a2, w2_ref[...], preferred_element_type=f32) + b2
        o_ref[rows, :] = (x1 + gb * y).astype(o_ref.dtype)


@jax.jit
def pallas_adaLN_cond__mha_block__dense_activation_squared_relu__prompt_kernel(
    A_x: jax.Array,
    A_wqkv: jax.Array,
    A_wo: jax.Array,
    B_x: jax.Array,
    B_w1: jax.Array,
    B_b1: jax.Array,
    B_w2: jax.Array,
    B_b2: jax.Array,
    c: jax.Array,
    w_mod: jax.Array,
):
    x2d = A_x.reshape(S, D)
    out = pl.pallas_call(
        _kernel,
        out_shape=jax.ShapeDtypeStruct((S, D), A_x.dtype),
        scratch_shapes=[
            pltpu.VMEM((S, D), jnp.bfloat16),
            pltpu.VMEM((D, S), jnp.bfloat16),
            pltpu.VMEM((D, S), jnp.bfloat16),
            pltpu.VMEM((D, S), jnp.bfloat16),
            pltpu.VMEM((H, 8, S), jnp.float32),
            pltpu.VMEM((8, 6 * D), jnp.float32),
        ],
        compiler_params=pltpu.CompilerParams(vmem_limit_bytes=100 * 1024 * 1024),
    )(x2d, A_wqkv, A_wo, B_w1, B_b1.reshape(1, F), B_w2, B_b2.reshape(1, D), c, w_mod)
    return out.reshape(1, S, D)
```

```python
import jax
import jax.numpy as jnp
import jax.experimental.pallas as pl
import jax.experimental.pallas.tpu as pltpu

S = 2048
D = 512
H = 32
DH = 16
F = 1792
EPS = 1e-5

LOG2E = 1.4426950408889634
QSCALE = (DH ** -0.5) * LOG2E

TQ = 512
CK = 128
UPB = 8
PIPE = 2
NQ = S // TQ
NU = H * NQ
NC = S // CK

RB = 512

LSUM_MIN = 2.0 ** -80

_NT = (((1,), (1,)), ((), ()))


def _layernorm(x):
    mu = jnp.mean(x, axis=-1, keepdims=True)
    xc = x - mu
    var = jnp.mean(xc * xc, axis=-1, keepdims=True)
    return xc * jax.lax.rsqrt(var + EPS)


def _kernel(x_hbm, wqkv_hbm, wo_hbm, w1_hbm, b1_hbm, w2_hbm, b2_hbm, c_hbm, wmod_hbm,
            o_hbm,
            x_ref, wqkv_ref, wo_ref, w1_ref, b1_ref, w2_ref, b2_ref, c_ref, wmod_ref, o_ref,
            k_scr, qt_scr, vt_scr, ot_scr, mb_scr, mod_scr, cs_scr, sems):
    f32 = jnp.float32
    bf16 = jnp.bfloat16
    NRB = S // RB

    cp_c = pltpu.make_async_copy(c_hbm, c_ref, sems.at[0])
    cp_wma = pltpu.make_async_copy(wmod_hbm.at[:, 0:2 * D], wmod_ref.at[:, 0:2 * D], sems.at[1])
    cp_wqkv = pltpu.make_async_copy(wqkv_hbm, wqkv_ref, sems.at[2])
    cp_x = [pltpu.make_async_copy(x_hbm.at[rb * RB:(rb + 1) * RB, :], x_ref.at[rb * RB:(rb + 1) * RB, :],
                                  sems.at[3 + rb]) for rb in range(NRB)]
    base = 3 + NRB
    cp_late = [
        pltpu.make_async_copy(wmod_hbm.at[:, 2 * D:6 * D], wmod_ref.at[:, 2 * D:6 * D], sems.at[base]),
        pltpu.make_async_copy(wo_hbm, wo_ref, sems.at[base + 1]),
        pltpu.make_async_copy(w1_hbm, w1_ref, sems.at[base + 2]),
        pltpu.make_async_copy(w2_hbm, w2_ref, sems.at[base + 3]),
        pltpu.make_async_copy(b1_hbm, b1_ref, sems.at[base + 4]),
        pltpu.make_async_copy(b2_hbm, b2_ref, sems.at[base + 5]),
    ]
    obase = base + 6
    cp_out = [pltpu.make_async_copy(o_ref.at[rb * RB:(rb + 1) * RB, :], o_hbm.at[rb * RB:(rb + 1) * RB, :],
                                    sems.at[obase + rb]) for rb in range(NRB)]
    cp_c.start()
    cp_wma.start()
    cp_x[0].start()
    cp_wqkv.start()

    cp_c.wait()
    cp_wma.wait()
    c = c_ref[...].astype(f32)
    sc = c * jax.nn.sigmoid(c)
    sc8 = jnp.broadcast_to(sc, (8, D)).astype(bf16)
    mod_scr[:, 0:2 * D] = jnp.dot(sc8, wmod_ref[:, 0:2 * D], preferred_element_type=f32)

    sa = mod_scr[0:1, 0 * D:1 * D]
    ca = mod_scr[0:1, 1 * D:2 * D]

    cp_x[0].wait()
    cp_wqkv.wait()
    for rb in range(1, NRB):
        cp_x[rb].start()
    wq_t = wqkv_ref[:, 0:D].astype(f32).T.astype(bf16)
    wv_t = wqkv_ref[:, 2 * D:3 * D].astype(f32).T.astype(bf16)
    gi = jax.lax.broadcasted_iota(jnp.int32, (H, D), 0)
    gj = jax.lax.broadcasted_iota(jnp.int32, (H, D), 1)
    gmat = jnp.where((gj // DH) == gi, 1.0, 0.0).astype(bf16)

    k2max = None
    q2_parts = []
    for rb in range(S // RB):
        rows = slice(rb * RB, (rb + 1) * RB)
        if rb == 1:
            for r2 in range(1, NRB):
                cp_x[r2].wait()
            for cp in cp_late:
                cp.start()
        xb = x_ref[rows, :].astype(f32)
        hb = (_layernorm(xb) * (1.0 + ca) + sa).astype(bf16)
        kb = jnp.dot(hb, wqkv_ref[:, D:2 * D], preferred_element_type=f32).astype(bf16)
        k_scr[rows, :] = kb
        qtb = (jax.lax.dot_general(wq_t, hb, _NT, preferred_element_type=f32) * QSCALE).astype(bf16)
        qt_scr[:, rows] = qtb
        vt_scr[:, rows] = jax.lax.dot_general(wv_t, hb, _NT, preferred_element_type=f32).astype(bf16)
        kf = kb.astype(f32)
        k2 = jax.lax.dot_general(gmat, (kf * kf).astype(bf16), _NT, preferred_element_type=f32)
        k2m = jnp.max(k2, axis=1, keepdims=True)
        k2max = k2m if k2max is None else jnp.maximum(k2max, k2m)
        qf = qtb.astype(f32)
        q2_parts.append(jnp.dot(gmat, (qf * qf).astype(bf16), preferred_element_type=f32))
    for rb in range(S // RB):
        mb = jnp.sqrt(q2_parts[rb] * k2max) * (1.0 + 2.0 ** -6)
        for h in range(H):
            mb_scr[h, :, rb * RB:(rb + 1) * RB] = jnp.broadcast_to(mb[h:h + 1, :], (8, RB))

    def masked_q(u, tq):
        nq = S // tq
        h = u // nq
        g = h // 8
        hh = h % 8
        goff = pl.multiple_of(g * 128, 128)
        qoff = pl.multiple_of((u % nq) * tq, tq)
        qt = qt_scr[pl.ds(goff, 128), pl.ds(qoff, tq)]
        row = jax.lax.broadcasted_iota(jnp.int32, (128, tq), 0)
        qm = jnp.where((row // DH) == hh, qt, jnp.zeros_like(qt))
        return h, goff, qoff, qm

    def unit_info(u):
        h, goff, qoff, qm = masked_q(u, TQ)
        m8 = mb_scr[h, :, pl.ds(qoff, TQ)]
        return goff, qm, m8

    def qk(c, goff, qm):
        kg = k_scr[c * CK:(c + 1) * CK, pl.ds(goff, 128)]
        return jnp.dot(kg, qm, preferred_element_type=f32)

    def softmax_pv(c, u, st, m8, acc, l):
        hoff = pl.multiple_of((u // NQ) * DH, DH)
        p = jnp.exp2(st.reshape(CK // 8, 8, TQ) - m8[None])
        ls = jnp.sum(p, axis=0)
        vt = vt_scr[pl.ds(hoff, DH), c * CK:(c + 1) * CK]
        ot = jnp.dot(vt, p.reshape(CK, TQ).astype(bf16), preferred_element_type=f32)
        return (ot if acc is None else acc + ot), (ls if l is None else l + ls)

    def finish(u, acc, l, lmin):
        hoff = pl.multiple_of((u // NQ) * DH, DH)
        qoff = pl.multiple_of((u % NQ) * TQ, TQ)
        lt = jnp.sum(l, axis=0, keepdims=True)
        ot_scr[pl.ds(hoff, DH), pl.ds(qoff, TQ)] = (acc / lt).astype(bf16)
        return jnp.minimum(lmin, lt)

    def attn_body(j, carry):
        cacc, cl, lmin = carry
        csts = [cs_scr[t] for t in range(PIPE)]
        uprev = jnp.maximum(j * UPB - 1, 0)
        hprev = uprev // NQ
        m8prev = mb_scr[hprev, :, pl.ds(pl.multiple_of((uprev % NQ) * TQ, TQ), TQ)]
        tiles = [(i, c) for i in range(UPB) for c in range(NC)]
        info = [unit_info(j * UPB + i) for i in range(UPB)]
        sts = {}
        accs = {i: (None, None) for i in range(UPB)}
        n = len(tiles)
        for t in range(n):
            i, c = tiles[t]
            sts[t] = qk(c, info[i][0], info[i][1])
            if t < PIPE:
                cacc, cl = softmax_pv(NC - PIPE + t, uprev, csts[t], m8prev, cacc, cl)
                if t == PIPE - 1:
                    lnew = finish(uprev, cacc, cl, lmin)
                    lmin = jnp.where(j > 0, lnew, lmin)
            else:
                i, c = tiles[t - PIPE]
                acc, l = accs[i]
                accs[i] = softmax_pv(c, j * UPB + i, sts.pop(t - PIPE), info[i][2], acc, l)
                if c == NC - 1:
                    lmin = finish(j * UPB + i, accs[i][0], accs[i][1], lmin)
        for t in range(PIPE):
            cs_scr[t] = sts[n - PIPE + t]
        return accs[UPB - 1][0], accs[UPB - 1][1], lmin

    cs_scr[...] = jnp.zeros((PIPE, CK, TQ), f32)
    init = (jnp.zeros((DH, TQ), f32), jnp.ones((8, TQ), f32), jnp.full((1, TQ), jnp.inf, f32))
    cacc, cl, lmin = jax.lax.fori_loop(0, NU // UPB, attn_body, init)
    csts = [cs_scr[t] for t in range(PIPE)]
    m8last = mb_scr[H - 1, :, S - TQ:S]
    for t in range(PIPE):
        cacc, cl = softmax_pv(NC - PIPE + t, NU - 1, csts[t], m8last, cacc, cl)
    lmin = finish(NU - 1, cacc, cl, lmin)
    safe = jnp.min(lmin) >= LSUM_MIN

    @pl.when(jnp.logical_not(safe))
    def _():
        tq = 128

        def exact_body(u, carry):
            h, goff, qoff, qm = masked_q(u, tq)
            hoff = pl.multiple_of(h * DH, DH)
            st = jnp.dot(k_scr[:, pl.ds(goff, 128)], qm, preferred_element_type=f32)
            m = jnp.max(st, axis=0, keepdims=True)
            p = jnp.exp2(st - m)
            lt = jnp.sum(p, axis=0, keepdims=True)
            ot = jnp.dot(vt_scr[pl.ds(hoff, DH), :], p.astype(bf16), preferred_element_type=f32)
            ot_scr[pl.ds(hoff, DH), pl.ds(qoff, tq)] = (ot / lt).astype(bf16)
            return carry

        jax.lax.fori_loop(0, H * (S // tq), exact_body, 0)

    for cp in cp_late:
        cp.wait()
    mod_scr[:, 2 * D:6 * D] = jnp.dot(sc8, wmod_ref[:, 2 * D:6 * D], preferred_element_type=f32)
    ga = mod_scr[0:1, 2 * D:3 * D]
    sb = mod_scr[0:1, 3 * D:4 * D]
    cb = mod_scr[0:1, 4 * D:5 * D]
    gb = mod_scr[0:1, 5 * D:6 * D]
    b1 = b1_ref[...].astype(f32).reshape(1, F)
    b2 = b2_ref[...].astype(f32).reshape(1, D)
    def mlp_body(rb, carry):
        r0 = pl.multiple_of(rb * RB, RB)
        rows = pl.ds(r0, RB)
        ob = ot_scr[:, rows].astype(f32).T.astype(bf16)
        attn = jnp.dot(ob, wo_ref[...], preferred_element_type=f32)
        x1 = x_ref[rows, :].astype(f32) + ga * attn
        h2 = (_layernorm(x1) * (1.0 + cb) + sb).astype(bf16)
        a = jnp.dot(h2, w1_ref[...], preferred_element_type=f32) + b1
        r = jnp.maximum(a, 0.0)
        a2 = (r * r).astype(bf16)
        y = jnp.dot(a2, w2_ref[...], preferred_element_type=f32) + b2
        o_ref[rows, :] = (x1 + gb * y).astype(o_ref.dtype)
        pltpu.make_async_copy(o_ref.at[rows, :], o_hbm.at[rows, :], sems.at[obase + rb]).start()
        return carry

    jax.lax.fori_loop(0, NRB, mlp_body, 0)
    for cp in cp_out:
        cp.wait()


@jax.jit
def pallas_adaLN_cond__mha_block__dense_activation_squared_relu__prompt_kernel(
    A_x: jax.Array,
    A_wqkv: jax.Array,
    A_wo: jax.Array,
    B_x: jax.Array,
    B_w1: jax.Array,
    B_b1: jax.Array,
    B_w2: jax.Array,
    B_b2: jax.Array,
    c: jax.Array,
    w_mod: jax.Array,
):
    x2d = A_x.reshape(S, D)
    out = pl.pallas_call(
        _kernel,
        out_shape=jax.ShapeDtypeStruct((S, D), A_x.dtype),
        in_specs=[pl.BlockSpec(memory_space=pl.ANY)] * 9,
        out_specs=pl.BlockSpec(memory_space=pl.ANY),
        scratch_shapes=[
            pltpu.VMEM((S, D), jnp.bfloat16),
            pltpu.VMEM((D, 3 * D), jnp.bfloat16),
            pltpu.VMEM((D, D), jnp.bfloat16),
            pltpu.VMEM((D, F), jnp.bfloat16),
            pltpu.VMEM((F,), jnp.bfloat16),
            pltpu.VMEM((F, D), jnp.bfloat16),
            pltpu.VMEM((D,), jnp.bfloat16),
            pltpu.VMEM((1, D), jnp.bfloat16),
            pltpu.VMEM((D, 6 * D), jnp.bfloat16),
            pltpu.VMEM((S, D), jnp.bfloat16),
            pltpu.VMEM((S, D), jnp.bfloat16),
            pltpu.VMEM((D, S), jnp.bfloat16),
            pltpu.VMEM((D, S), jnp.bfloat16),
            pltpu.VMEM((D, S), jnp.bfloat16),
            pltpu.VMEM((H, 8, S), jnp.float32),
            pltpu.VMEM((8, 6 * D), jnp.float32),
            pltpu.VMEM((PIPE, CK, TQ), jnp.float32),
            pltpu.SemaphoreType.DMA((3 + 2 * (S // RB) + 6,)),
        ],
        compiler_params=pltpu.CompilerParams(vmem_limit_bytes=100 * 1024 * 1024),
    )(x2d, A_wqkv, A_wo, B_w1, B_b1, B_w2, B_b2, c, w_mod)
    return out.reshape(1, S, D)
```

```python
import jax
import jax.numpy as jnp
import jax.experimental.pallas as pl
import jax.experimental.pallas.tpu as pltpu

S = 2048
D = 512
H = 32
DH = 16
F = 1792
EPS = 1e-5

LOG2E = 1.4426950408889634
QSCALE = (DH ** -0.5) * LOG2E

TQ = 512
CK = 128
UPB = 8
PIPE = 2
NQ = S // TQ
NU = H * NQ
NC = S // CK

RB = 512
SB = 256
OPB = 1

LSUM_MIN = 2.0 ** -80
LSUM_MAX = 2.0 ** 20

_NT = (((1,), (1,)), ((), ()))


def _layernorm(x):
    mu = jnp.mean(x, axis=-1, keepdims=True)
    xc = x - mu
    var = jnp.mean(xc * xc, axis=-1, keepdims=True)
    return xc * jax.lax.rsqrt(var + EPS)


def _kernel(x_hbm, wqkv_hbm, wo_hbm, w1_hbm, b1_hbm, w2_hbm, b2_hbm, c_hbm, wmod_hbm,
            o_hbm,
            x_ref, wqkv_ref, wo_ref, w1_ref, b1_ref, w2_ref, b2_ref, c_ref, wmod_ref, o_ref,
            k_scr, qt_scr, vt_scr, ot_scr, mb_scr, mod_scr, cs_scr, sems):
    f32 = jnp.float32
    bf16 = jnp.bfloat16
    NRB = S // RB

    cp_c = pltpu.make_async_copy(c_hbm, c_ref, sems.at[0])
    cp_wma = pltpu.make_async_copy(wmod_hbm.at[:, 0:2 * D], wmod_ref.at[:, 0:2 * D], sems.at[1])
    nsem_extra = 3 + 2 * NRB + 6
    cp_wk = pltpu.make_async_copy(wqkv_hbm.at[:, D:2 * D], wqkv_ref.at[:, D:2 * D], sems.at[2])
    cp_wq = pltpu.make_async_copy(wqkv_hbm.at[:, 0:D], wqkv_ref.at[:, 0:D], sems.at[nsem_extra])
    cp_wv = pltpu.make_async_copy(wqkv_hbm.at[:, 2 * D:3 * D], wqkv_ref.at[:, 2 * D:3 * D], sems.at[nsem_extra + 1])
    cp_x = [pltpu.make_async_copy(x_hbm.at[rb * RB:(rb + 1) * RB, :], x_ref.at[rb * RB:(rb + 1) * RB, :],
                                  sems.at[3 + rb]) for rb in range(NRB)]
    base = 3 + NRB
    cp_late = [
        pltpu.make_async_copy(wmod_hbm.at[:, 2 * D:6 * D], wmod_ref.at[:, 2 * D:6 * D], sems.at[base]),
        pltpu.make_async_copy(wo_hbm, wo_ref, sems.at[base + 1]),
        pltpu.make_async_copy(w1_hbm, w1_ref, sems.at[base + 2]),
        pltpu.make_async_copy(w2_hbm, w2_ref, sems.at[base + 3]),
        pltpu.make_async_copy(b1_hbm, b1_ref, sems.at[base + 4]),
        pltpu.make_async_copy(b2_hbm, b2_ref, sems.at[base + 5]),
    ]
    obase = base + 6
    cp_out = [pltpu.make_async_copy(o_ref.at[rb * RB:(rb + 1) * RB, :], o_hbm.at[rb * RB:(rb + 1) * RB, :],
                                    sems.at[obase + rb]) for rb in range(NRB)]
    cp_c.start()
    cp_wma.start()
    cp_x[0].start()
    cp_wk.start()
    cp_wq.start()
    cp_wv.start()

    cp_c.wait()
    cp_wma.wait()
    c = c_ref[...].astype(f32)
    sc = c * jax.nn.sigmoid(c)
    sc8 = jnp.broadcast_to(sc, (8, D)).astype(bf16)
    mod_scr[:, 0:2 * D] = jnp.dot(sc8, wmod_ref[:, 0:2 * D], preferred_element_type=f32)

    sa = mod_scr[0:1, 0 * D:1 * D]
    ca = mod_scr[0:1, 1 * D:2 * D]

    cp_x[0].wait()
    cp_wk.wait()
    gi = jax.lax.broadcasted_iota(jnp.int32, (H, D), 0)
    gj = jax.lax.broadcasted_iota(jnp.int32, (H, D), 1)
    gmat = jnp.where((gj // DH) == gi, 1.0, 0.0).astype(bf16)

    k2max = None
    q2_parts = []
    for rb in range(NRB):
        rows = slice(rb * RB, (rb + 1) * RB)
        xb = x_ref[rows, :].astype(f32)
        hb = (_layernorm(xb) * (1.0 + ca) + sa).astype(bf16)
        kb = jnp.dot(hb, wqkv_ref[:, D:2 * D], preferred_element_type=f32).astype(bf16)
        k_scr[rows, :] = kb
        if rb == 0:
            cp_wq.wait()
            cp_wv.wait()
            for r2 in range(1, NRB):
                cp_x[r2].start()
            wq_t = wqkv_ref[:, 0:D].astype(f32).T.astype(bf16)
            wv_t = wqkv_ref[:, 2 * D:3 * D].astype(f32).T.astype(bf16)
        qtb = (jax.lax.dot_general(wq_t, hb, _NT, preferred_element_type=f32) * QSCALE).astype(bf16)
        qt_scr[:, rows] = qtb
        if rb == 0:
            for r2 in range(1, NRB):
                cp_x[r2].wait()
            for cp in cp_late:
                cp.start()
        vt_scr[:, rows] = jax.lax.dot_general(wv_t, hb, _NT, preferred_element_type=f32).astype(bf16)
        kf = kb.astype(f32)
        k2 = jax.lax.dot_general(gmat, (kf * kf).astype(bf16), _NT, preferred_element_type=f32)
        k2m = jnp.max(k2, axis=1, keepdims=True)
        k2max = k2m if k2max is None else jnp.maximum(k2max, k2m)
        qf = qtb.astype(f32)
        q2_parts.append(jnp.dot(gmat, (qf * qf).astype(bf16), preferred_element_type=f32))
    cp_late[0].wait()
    mod_scr[:, 2 * D:6 * D] = jnp.dot(sc8, wmod_ref[:, 2 * D:6 * D], preferred_element_type=f32)
    for rb in range(S // RB):
        mb = jnp.sqrt(q2_parts[rb] * k2max) * (1.0 + 2.0 ** -6)
        for h in range(H):
            mb_scr[h, :, rb * RB:(rb + 1) * RB] = jnp.broadcast_to(mb[h:h + 1, :], (8, RB))

    def masked_q(u, tq):
        nq = S // tq
        h = u // nq
        g = h // 8
        hh = h % 8
        goff = pl.multiple_of(g * 128, 128)
        qoff = pl.multiple_of((u % nq) * tq, tq)
        qt = qt_scr[pl.ds(goff, 128), pl.ds(qoff, tq)]
        row = jax.lax.broadcasted_iota(jnp.int32, (128, tq), 0)
        qm = jnp.where((row // DH) == hh, qt, jnp.zeros_like(qt))
        return h, goff, qoff, qm

    def unit_info(u):
        h, goff, qoff, qm = masked_q(u, TQ)
        m8 = mb_scr[h, :, pl.ds(qoff, TQ)]
        return goff, qm, m8

    def qk(c, goff, qm):
        kg = k_scr[c * CK:(c + 1) * CK, pl.ds(goff, 128)]
        return jnp.dot(kg, qm, preferred_element_type=f32)

    def softmax_pv(c, u, st, m8, acc, l):
        hoff = pl.multiple_of((u // NQ) * DH, DH)
        p = jnp.exp2(st.reshape(CK // 8, 8, TQ) - m8[None])
        ls = jnp.sum(p, axis=0)
        vt = vt_scr[pl.ds(hoff, DH), c * CK:(c + 1) * CK]
        ot = jnp.dot(vt, p.reshape(CK, TQ).astype(bf16), preferred_element_type=f32)
        return (ot if acc is None else acc + ot), (ls if l is None else l + ls)

    def finish(u, acc, l, bad):
        hoff = pl.multiple_of((u // NQ) * DH, DH)
        qoff = pl.multiple_of((u % NQ) * TQ, TQ)
        lt = jnp.sum(l, axis=0, keepdims=True)
        ot_scr[pl.ds(hoff, DH), pl.ds(qoff, TQ)] = (acc / lt).astype(bf16)
        ok = jnp.logical_and(lt >= LSUM_MIN, lt <= LSUM_MAX)
        return jnp.maximum(bad, jnp.where(ok, 0.0, 1.0))

    def attn_body(j, carry):
        cacc, cl, bad = carry
        csts = [cs_scr[t] for t in range(PIPE)]
        uprev = jnp.maximum(j * UPB - 1, 0)
        hprev = uprev // NQ
        m8prev = mb_scr[hprev, :, pl.ds(pl.multiple_of((uprev % NQ) * TQ, TQ), TQ)]
        tiles = [(i, c) for i in range(UPB) for c in range(NC)]
        info = [unit_info(j * UPB + i) for i in range(UPB)]
        sts = {}
        accs = {i: (None, None) for i in range(UPB)}
        n = len(tiles)
        for t in range(n):
            i, c = tiles[t]
            sts[t] = qk(c, info[i][0], info[i][1])
            if t < PIPE:
                cacc, cl = softmax_pv(NC - PIPE + t, uprev, csts[t], m8prev, cacc, cl)
                if t == PIPE - 1:
                    bnew = finish(uprev, cacc, cl, bad)
                    bad = jnp.where(j > 0, bnew, bad)
            else:
                i, c = tiles[t - PIPE]
                acc, l = accs[i]
                accs[i] = softmax_pv(c, j * UPB + i, sts.pop(t - PIPE), info[i][2], acc, l)
                if c == NC - 1:
                    bad = finish(j * UPB + i, accs[i][0], accs[i][1], bad)
        for t in range(PIPE):
            cs_scr[t] = sts[n - PIPE + t]
        return accs[UPB - 1][0], accs[UPB - 1][1], bad

    cs_scr[...] = jnp.zeros((PIPE, CK, TQ), f32)
    init = (jnp.zeros((DH, TQ), f32), jnp.ones((8, TQ), f32), jnp.zeros((1, TQ), f32))
    cacc, cl, bad = jax.lax.fori_loop(0, NU // UPB, attn_body, init)
    csts = [cs_scr[t] for t in range(PIPE)]
    m8last = mb_scr[H - 1, :, S - TQ:S]
    for t in range(PIPE):
        cacc, cl = softmax_pv(NC - PIPE + t, NU - 1, csts[t], m8last, cacc, cl)
    bad = finish(NU - 1, cacc, cl, bad)
    unsafe = jnp.max(bad) > 0.0

    @pl.when(unsafe)
    def _():
        tq = 128

        def exact_body(u, carry):
            h, goff, qoff, qm = masked_q(u, tq)
            hoff = pl.multiple_of(h * DH, DH)
            st = jnp.dot(k_scr[:, pl.ds(goff, 128)], qm, preferred_element_type=f32)
            m = jnp.max(st, axis=0, keepdims=True)
            p = jnp.exp2(st - m)
            lt = jnp.sum(p, axis=0, keepdims=True)
            ot = jnp.dot(vt_scr[pl.ds(hoff, DH), :], p.astype(bf16), preferred_element_type=f32)
            ot_scr[pl.ds(hoff, DH), pl.ds(qoff, tq)] = (ot / lt).astype(bf16)
            return carry

        jax.lax.fori_loop(0, H * (S // tq), exact_body, 0)

    for cp in cp_late[1:]:
        cp.wait()
    ga = mod_scr[0:1, 2 * D:3 * D]
    sb = mod_scr[0:1, 3 * D:4 * D]
    cb = mod_scr[0:1, 4 * D:5 * D]
    gb = mod_scr[0:1, 5 * D:6 * D]
    b1 = b1_ref[...].astype(f32).reshape(1, F)
    b2 = b2_ref[...].astype(f32).reshape(1, D)

    def pre(r0):
        rows = pl.ds(r0, SB)
        ob = ot_scr[:, rows].astype(f32).T.astype(bf16)
        attn = jnp.dot(ob, wo_ref[...], preferred_element_type=f32)
        x1 = x_ref[rows, :].astype(f32) + ga * attn
        h2 = (_layernorm(x1) * (1.0 + cb) + sb).astype(bf16)
        return x1, h2

    def mlp(r0, x1, h2):
        a = jnp.dot(h2, w1_ref[...], preferred_element_type=f32) + b1
        r = jnp.maximum(a, 0.0)
        a2 = (r * r).astype(bf16)
        y = jnp.dot(a2, w2_ref[...], preferred_element_type=f32) + b2
        o_ref[pl.ds(r0, SB), :] = (x1 + gb * y).astype(o_ref.dtype)

    def mlp_body(it, carry):
        base_row = it * (RB * OPB)
        offs = [pl.multiple_of(base_row + i * SB, SB) for i in range(RB * OPB // SB)]
        nxt = pre(offs[0])
        for i in range(len(offs)):
            cur = nxt
            if i + 1 < len(offs):
                nxt = pre(offs[i + 1])
            mlp(offs[i], *cur)
            if ((i + 1) * SB) % RB == 0:
                rb = it * OPB + ((i + 1) * SB) // RB - 1
                rows = pl.ds(pl.multiple_of(rb * RB, RB), RB)
                pltpu.make_async_copy(o_ref.at[rows, :], o_hbm.at[rows, :], sems.at[obase + rb]).start()
        return carry

    jax.lax.fori_loop(0, NRB // OPB, mlp_body, 0)
    for cp in cp_out:
        cp.wait()


@jax.jit
def pallas_adaLN_cond__mha_block__dense_activation_squared_relu__prompt_kernel(
    A_x: jax.Array,
    A_wqkv: jax.Array,
    A_wo: jax.Array,
    B_x: jax.Array,
    B_w1: jax.Array,
    B_b1: jax.Array,
    B_w2: jax.Array,
    B_b2: jax.Array,
    c: jax.Array,
    w_mod: jax.Array,
):
    x2d = A_x.reshape(S, D)
    out = pl.pallas_call(
        _kernel,
        out_shape=jax.ShapeDtypeStruct((S, D), A_x.dtype),
        in_specs=[pl.BlockSpec(memory_space=pl.ANY)] * 9,
        out_specs=pl.BlockSpec(memory_space=pl.ANY),
        scratch_shapes=[
            pltpu.VMEM((S, D), jnp.bfloat16),
            pltpu.VMEM((D, 3 * D), jnp.bfloat16),
            pltpu.VMEM((D, D), jnp.bfloat16),
            pltpu.VMEM((D, F), jnp.bfloat16),
            pltpu.VMEM((F,), jnp.bfloat16),
            pltpu.VMEM((F, D), jnp.bfloat16),
            pltpu.VMEM((D,), jnp.bfloat16),
            pltpu.VMEM((1, D), jnp.bfloat16),
            pltpu.VMEM((D, 6 * D), jnp.bfloat16),
            pltpu.VMEM((S, D), jnp.bfloat16),
            pltpu.VMEM((S, D), jnp.bfloat16),
            pltpu.VMEM((D, S), jnp.bfloat16),
            pltpu.VMEM((D, S), jnp.bfloat16),
            pltpu.VMEM((D, S), jnp.bfloat16),
            pltpu.VMEM((H, 8, S), jnp.float32),
            pltpu.VMEM((8, 6 * D), jnp.float32),
            pltpu.VMEM((PIPE, CK, TQ), jnp.float32),
            pltpu.SemaphoreType.DMA((3 + 2 * (S // RB) + 6 + 2,)),
        ],
        compiler_params=pltpu.CompilerParams(vmem_limit_bytes=100 * 1024 * 1024),
    )(x2d, A_wqkv, A_wo, B_w1, B_b1, B_w2, B_b2, c, w_mod)
    return out.reshape(1, S, D)
```
